```python
import jax
import jax.numpy as jnp

def _softmax(x, axis=-1):
    return jax.nn.softmax(x, axis=axis)

def _gelu(x):
    return jax.nn.gelu(x, approximate=True)

def _silu(x):
    return jax.nn.silu(x)

def _sigmoid(x):
    return jax.nn.sigmoid(x)

def _layernorm(x, axis=-1, eps=1e-05):
    m = jnp.mean(x, axis=axis, keepdims=True)
    v = jnp.var(x, axis=axis, keepdims=True)
    return (x - m) / jnp.sqrt(v + eps)

def _scatter_add(tgt, idx, src, axis=0):
    return tgt.at[idx].add(src)

def _segment_sum(src, seg, n):
    return jax.ops.segment_sum(src, seg, n)

class _Rng:

    def __init__(self, key):
        self._k = key

    def _next(self):
        self._k, sub = jax.random.split(self._k)
        return sub

    def normal(self, shape):
        return jax.random.normal(self._next(), shape, dtype=jnp.bfloat16)

    def randint(self, lo, hi, shape):
        return jax.random.randint(self._next(), shape, lo, hi, dtype=jnp.int32)

    def uniform(self, shape, lo=0.0, hi=1.0):
        return jax.random.uniform(self._next(), shape, jnp.bfloat16, lo, hi)

    def permutation(self, n):
        return jax.random.permutation(self._next(), n)
kernel_name = 'adaLN_cond__compressed_kv_cla__glu_gated_geglu__decode'

def setup_inputs():
    _rng = _Rng(jax.random.key(int.from_bytes(__import__("os").urandom(4), "little")))
    _w = lambda a: (lambda t: t.astype(jnp.bfloat16) if jnp.issubdtype(t.dtype, jnp.floating) else t)(jnp.asarray(a))

    def _A_setup():
        B, H, Sq, Sk, D, M = (1, 32, 1, 32768, 128, 512)
        Dc = 4 * D
        return {'x': _w((lambda *s: _rng.normal(s) * 0.05)(B, Sq, M)), 'c_kv': _w((lambda *s: _rng.normal(s) * 0.05)(B, Sk, Dc)), 'w_q': _w((lambda *s: _rng.normal(s) * 0.05)(M, H, D) * M ** (-0.5)), 'w_uk': _w((lambda *s: _rng.normal(s) * 0.05)(Dc, H, D) * Dc ** (-0.5)), 'w_uv': _w((lambda *s: _rng.normal(s) * 0.05)(Dc, H, D) * Dc ** (-0.5)), 'w_o': _w((lambda *s: _rng.normal(s) * 0.05)(H, D, M) * (H * D) ** (-0.5))}
    _A_in = _A_setup()

    def _B_setup():
        B, S, Dm, Df = (1, 1, 512, 1792)
        return {'x': _w((lambda *s: _rng.normal(s) * 0.05)(B, S, Dm)), 'w_gate': _w((lambda *s: _rng.normal(s) * 0.05)(Dm, Df) * Dm ** (-0.5)), 'w_up': _w((lambda *s: _rng.normal(s) * 0.05)(Dm, Df) * Dm ** (-0.5)), 'w_down': _w((lambda *s: _rng.normal(s) * 0.05)(Df, Dm) * Df ** (-0.5))}
    _B_in = _B_setup()
    return {'A_x': _A_in['x'], 'A_c_kv': _A_in['c_kv'], 'A_w_q': _A_in['w_q'], 'A_w_uk': _A_in['w_uk'], 'A_w_uv': _A_in['w_uv'], 'A_w_o': _A_in['w_o'], 'B_x': _B_in['x'], 'B_w_gate': _B_in['w_gate'], 'B_w_up': _B_in['w_up'], 'B_w_down': _B_in['w_down'], 'c': _w((lambda *s: _rng.normal(s) * 0.05)(1, 512)), 'w_mod': _w((lambda *s: _rng.normal(s) * 0.05)(512, 6 * 512) * 512 ** (-0.5))}

def reference(A_x, A_c_kv, A_w_q, A_w_uk, A_w_uv, A_w_o, B_x, B_w_gate, B_w_up, B_w_down, c, w_mod):

    def _A_ref(x, c_kv, w_q, w_uk, w_uv, w_o):
        B, Sq, M = (x.shape[0], x.shape[1], x.shape[2])
        Sk = c_kv.shape[1]
        H, D = (w_q.shape[1], w_q.shape[2])
        q = jnp.einsum('bqm,mhd->bhqd', x, w_q)
        k = jnp.einsum('bkc,chd->bhkd', c_kv, w_uk)
        v = jnp.einsum('bkc,chd->bhkd', c_kv, w_uv)
        scores = jnp.einsum('bhqd,bhkd->bhqk', q, k) * D ** (-0.5)
        off = Sk - Sq
        qi = jnp.arange(Sq)[:, None]
        kj = jnp.arange(Sk)[None, :]
        cmask = kj <= qi + off
        scores = jnp.where(cmask[None, None], scores, -1000000000.0)
        p = _softmax(scores, axis=-1)
        ctx = jnp.einsum('bhqk,bhkd->bhqd', p, v)
        return jnp.einsum('bhqd,hdm->bqm', ctx, w_o)

    def _B_ref(x, w_gate, w_up, w_down):
        g = jnp.einsum('bsd,df->bsf', x, w_gate)
        u = jnp.einsum('bsd,df->bsf', x, w_up)
        h = _gelu(g) * u
        return jnp.einsum('bsf,fd->bsd', h, w_down)
    x = A_x
    mod = (_silu(c) @ w_mod).reshape(c.shape[0], 6, 1, -1)
    sa, ca, ga, sb, cb, gb = (mod[:, 0].copy(), mod[:, 1].copy(), mod[:, 2].copy(), mod[:, 3].copy(), mod[:, 4].copy(), mod[:, 5].copy())
    h = _layernorm(x, axis=-1) * (1 + ca) + sa
    x = x + ga * _A_ref(h, A_c_kv, A_w_q, A_w_uk, A_w_uv, A_w_o)
    h = _layernorm(x, axis=-1) * (1 + cb) + sb
    x = x + gb * _B_ref(h, B_w_gate, B_w_up, B_w_down)
    return x
```

```python
import functools
import jax
import jax.numpy as jnp
from jax.experimental import pallas as pl
from jax.experimental.pallas import tpu as pltpu

F32 = jnp.float32
BF16 = jnp.bfloat16

H, D, M, SK, DC, DF = 32, 128, 512, 32768, 512, 1792


def build(n_ckv=8, tk=2048, wd_last=256, unroll_h=4, unroll_t=2):
    ckv_chunk = SK // n_ckv
    S_MOD, S_X, S_C, S_Q, S_UK = 0, 1, 2, 3, 4
    S_CKV = 5
    S_UV = S_CKV + n_ckv
    S_O, S_G, S_U, S_D0, S_D1 = S_UV + 1, S_UV + 2, S_UV + 3, S_UV + 4, S_UV + 5
    NSEM = S_D1 + 1
    wd0 = DF - wd_last

    def kern(x_h, ckv_h, wq_h, wuk_h, wuv_h, wo_h, wg_h, wu_h, wd_h, c_h, wmod_h,
             o_ref,
             x_v, ckv_v, wq_v, wuk_v, wuv_v, wo_v, wg_v, wu_v, wd_v, c_v, wmod_v,
             mod_v, sems):
        def whole(src, dst, s):
            return pltpu.make_async_copy(src, dst, sems.at[s])

        def ckv_cp(i):
            sl = pl.ds(pl.multiple_of(i * ckv_chunk, ckv_chunk), ckv_chunk)
            return pltpu.make_async_copy(ckv_h.at[sl], ckv_v.at[sl], sems.at[S_CKV + i])

        cp_mod = whole(wmod_h, wmod_v, S_MOD)
        cp_x = whole(x_h, x_v, S_X)
        cp_c = whole(c_h, c_v, S_C)
        cp_q = whole(wq_h, wq_v, S_Q)
        cp_uk = whole(wuk_h, wuk_v, S_UK)
        cp_uv = whole(wuv_h, wuv_v, S_UV)
        cp_o = whole(wo_h, wo_v, S_O)
        cp_g = whole(wg_h, wg_v, S_G)
        cp_u = whole(wu_h, wu_v, S_U)
        cp_d0 = pltpu.make_async_copy(wd_h.at[pl.ds(0, wd0)], wd_v.at[pl.ds(0, wd0)], sems.at[S_D0])
        cp_d1 = pltpu.make_async_copy(wd_h.at[pl.ds(wd0, wd_last)], wd_v.at[pl.ds(wd0, wd_last)], sems.at[S_D1])

        cp_mod.start(); cp_x.start(); cp_c.start(); cp_q.start(); cp_uk.start()
        for i in range(n_ckv):
            ckv_cp(i).start()
        cp_uv.start(); cp_o.start(); cp_g.start(); cp_u.start(); cp_d0.start(); cp_d1.start()

        cp_mod.wait(); cp_x.wait(); cp_c.wait()
        cf = c_v[...].astype(F32)
        sc = cf * jax.nn.sigmoid(cf)
        sc16 = jnp.broadcast_to(sc, (16, M)).astype(BF16)

        def mod_body(j, _):
            off = pl.multiple_of(j * M, M)
            mod_v[j] = jnp.dot(sc16, wmod_v[:, pl.ds(off, M)], preferred_element_type=F32)[0:8]
            return 0
        jax.lax.fori_loop(0, 6, mod_body, 0)

        def modrow(j):
            return mod_v[j][0:1, :].astype(BF16).astype(F32)

        def layernorm(v):
            mu = jnp.mean(v, axis=-1, keepdims=True)
            ce = v - mu
            var = jnp.mean(ce * ce, axis=-1, keepdims=True)
            return ce * jax.lax.rsqrt(var + 1e-5)

        xf = x_v[...].astype(F32)
        h1 = layernorm(xf) * (1.0 + modrow(1)) + modrow(0)

        row128 = jax.lax.broadcasted_iota(jnp.int32, (128, 128), 0)
        col128 = jax.lax.broadcasted_iota(jnp.int32, (128, 128), 1)
        row32 = jax.lax.broadcasted_iota(jnp.int32, (32, 128), 0)
        col32 = jax.lax.broadcasted_iota(jnp.int32, (32, 128), 1)

        def rep_tile(t):
            return jnp.where(row128 == 4 * t + (col128 >> 5), 1.0, 0.0).astype(BF16)

        def rep_tile_T(t):
            return jnp.where(col128 == 4 * t + (row128 >> 5), 1.0, 0.0).astype(BF16)

        def head_mask(v):
            return jnp.where((col32 & 31) == row32, v, 0.0)

        def expand_contract(lhs_stack, w_v):
            def body(t, acc):
                e = jnp.dot(lhs_stack, rep_tile(t), preferred_element_type=F32)
                for i in range(4):
                    a = head_mask(e[32 * i:32 * (i + 1)]).astype(BF16)
                    off = pl.multiple_of(4096 * i + 128 * t, 128)
                    acc = acc + jnp.dot(a, w_v[pl.ds(off, 128), :], preferred_element_type=F32)
                return acc
            return jax.lax.fori_loop(0, 32, body, jnp.zeros((H, D), F32), unroll=unroll_t)

        h1b = jnp.broadcast_to(h1, (32, M)).astype(BF16)
        h1_stack = jnp.concatenate([h1b[:, 128 * i:128 * (i + 1)] for i in range(4)], axis=0)
        cp_q.wait()
        q = expand_contract(h1_stack, wq_v)
        qb = q.astype(BF16)

        cp_uk.wait()
        scale = D ** -0.5

        def ql_body(t, acc):
            zs = []
            for i in range(4):
                off = pl.multiple_of(4096 * i + 128 * t, 128)
                tt = jax.lax.dot_general(qb, wuk_v[pl.ds(off, 128), :], (((1,), (1,)), ((), ())),
                                         preferred_element_type=F32)
                zs.append(head_mask(tt * scale).astype(BF16))
            z = jnp.concatenate(zs, axis=0)
            return acc + jnp.dot(z, rep_tile_T(t), preferred_element_type=F32)
        ql_stack = jax.lax.fori_loop(0, 32, ql_body, jnp.zeros((128, 128), F32), unroll=unroll_t)
        ql = jnp.concatenate([ql_stack[32 * i:32 * (i + 1)] for i in range(4)], axis=1).astype(BF16)

        nsub = ckv_chunk // tk

        def sub_body(off, carry):
            m, l, acc = carry
            cc = ckv_v[pl.ds(off, tk), :]
            s = jax.lax.dot_general(ql, cc, (((1,), (1,)), ((), ())), preferred_element_type=F32)
            mn = jnp.maximum(m, jnp.max(s, axis=1, keepdims=True))
            a = jnp.exp(m - mn)
            p = jnp.exp(s - mn)
            l = a * l + jnp.sum(p, axis=1, keepdims=True)
            acc = a * acc + jnp.dot(p.astype(BF16), cc, preferred_element_type=F32)
            return mn, l, acc

        def chunk_body(i, carry):
            ckv_cp(i).wait()
            if nsub == 1:
                return sub_body(pl.multiple_of(i * ckv_chunk, tk), carry)
            return jax.lax.fori_loop(
                0, nsub, lambda j, cr: sub_body(pl.multiple_of(i * ckv_chunk + j * tk, tk), cr), carry)

        m, l, acc = jax.lax.fori_loop(
            0, n_ckv, chunk_body,
            (jnp.full((H, 1), -1e30, F32), jnp.zeros((H, 1), F32), jnp.zeros((H, DC), F32)))
        ob = (acc / l).astype(BF16)
        ob_stack = jnp.concatenate([ob[:, 128 * i:128 * (i + 1)] for i in range(4)], axis=0)

        cp_uv.wait()
        ctx = expand_contract(ob_stack, wuv_v)

        cp_o.wait()

        def o_body(hh, acc):
            a = jnp.where(row32 == hh, ctx, 0.0).astype(BF16)
            off = pl.multiple_of(hh * 128, 128)
            return acc + jnp.dot(a, wo_v[pl.ds(off, 128), :], preferred_element_type=F32)
        oacc = jax.lax.fori_loop(0, H, o_body, jnp.zeros((H, M), F32), unroll=unroll_h)
        attn = jnp.sum(oacc, axis=0, keepdims=True)
        x1 = xf + modrow(2) * attn
        h2 = layernorm(x1) * (1.0 + modrow(4)) + modrow(3)
        h2b = jnp.broadcast_to(h2, (16, M)).astype(BF16)

        cp_g.wait()
        g = jnp.dot(h2b, wg_v[...], preferred_element_type=F32)[0:8]
        cp_u.wait()
        u = jnp.dot(h2b, wu_v[...], preferred_element_type=F32)[0:8]
        act = jax.nn.gelu(g, approximate=True) * u
        act16 = jnp.concatenate([act, act], axis=0).astype(BF16)
        cp_d0.wait()
        y = jnp.dot(act16[:, :wd0], wd_v[pl.ds(0, wd0), :], preferred_element_type=F32)
        cp_d1.wait()
        y = y + jnp.dot(act16[:, wd0:], wd_v[pl.ds(wd0, wd_last), :], preferred_element_type=F32)
        o_ref[...] = (x1 + modrow(5) * y[0:1]).astype(BF16)

    hbm = pl.BlockSpec(memory_space=pltpu.HBM)

    @jax.jit
    def f(A_x, A_c_kv, A_w_q, A_w_uk, A_w_uv, A_w_o, B_x, B_w_gate, B_w_up, B_w_down, c, w_mod):
        out = pl.pallas_call(
            kern,
            out_shape=jax.ShapeDtypeStruct((1, M), BF16),
            in_specs=[hbm] * 11,
            out_specs=pl.BlockSpec(memory_space=pltpu.VMEM),
            scratch_shapes=[
                pltpu.VMEM((1, M), BF16), pltpu.VMEM((SK, DC), BF16),
                pltpu.VMEM((M * H, D), BF16), pltpu.VMEM((DC * H, D), BF16), pltpu.VMEM((DC * H, D), BF16),
                pltpu.VMEM((H * D, M), BF16), pltpu.VMEM((M, DF), BF16), pltpu.VMEM((M, DF), BF16),
                pltpu.VMEM((DF, M), BF16), pltpu.VMEM((1, M), BF16), pltpu.VMEM((M, 6 * M), BF16),
                pltpu.VMEM((6, 8, M), F32), pltpu.SemaphoreType.DMA((NSEM,)),
            ],
            compiler_params=pltpu.CompilerParams(vmem_limit_bytes=100 * 1024 * 1024),
        )(A_x.reshape(1, M), A_c_kv.reshape(SK, DC), A_w_q.reshape(M * H, D), A_w_uk.reshape(DC * H, D),
          A_w_uv.reshape(DC * H, D), A_w_o.reshape(H * D, M), B_w_gate, B_w_up, B_w_down, c, w_mod)
        return out.reshape(1, 1, M)
    return f


_kernel = build()


@jax.jit
def pallas_adaLN_cond__compressed_kv_cla__glu_gated_geglu__decode_kernel(
    A_x, A_c_kv, A_w_q, A_w_uk, A_w_uv, A_w_o, B_x, B_w_gate, B_w_up, B_w_down, c, w_mod,
):
    return _kernel(A_x, A_c_kv, A_w_q, A_w_uk, A_w_uv, A_w_o, B_x, B_w_gate, B_w_up, B_w_down, c, w_mod)
```

```python
import jax
import jax.numpy as jnp
from jax.experimental import pallas as pl
from jax.experimental.pallas import tpu as pltpu

F32 = jnp.float32
BF16 = jnp.bfloat16

H, D, M, DC, DF = 32, 128, 512, 512, 1792
SK = 32768
N_CKV = 16
N_WD, WD_CH = 6, 256
WD_A, WD_V = 128, 128
RING = 4
UNROLL_T, UNROLL_H = 8, 8


def _make(sk=SK, n_ckv=N_CKV, interpret=False):
    tk = sk // n_ckv
    off_a = N_WD * WD_CH
    off_v = off_a + WD_A
    assert tk * n_ckv == sk and off_v + WD_V == DF and n_ckv >= RING and N_WD >= RING

    j_mod, j_q, j_uk, j_ckv = 0, 1, 2, 3
    j_uv = j_ckv + n_ckv
    j_o, j_g, j_u, j_d = j_uv + 1, j_uv + 2, j_uv + 3, j_uv + 4
    j_a = j_d + N_WD
    j_v = j_a + 1
    n_j = j_v + 1

    def kernel(x_h, ckv_h, wq_h, wuk_h, wuv_h, wo_h, wg_h, wu_h, wd_h, c_h, wmod_h,
               o_ref,
               x_v, ckv_v, wq_v, wuk_v, wuv_v, wo_v, wg_v, wu_v, wd_v, c_v, wmod_v,
               mod_v, act_v, sems):
        mk = pltpu.make_async_copy

        def ckv_copy(i):
            sl = pl.ds(pl.multiple_of(i * tk, tk), tk)
            return mk(ckv_h.at[sl], ckv_v.at[sl], sems.at[(j_ckv + i) % RING])

        def wd_copy(i):
            sl = pl.ds(pl.multiple_of(i * WD_CH, WD_CH), WD_CH)
            return mk(wd_h.at[sl], wd_v.at[sl], sems.at[(j_d + i) % RING])

        def copies(j):
            s = sems.at[j % RING]
            if j == j_mod:
                return [mk(wmod_h, wmod_v, s), mk(x_h, x_v, s), mk(c_h, c_v, s)]
            if j == j_q:
                return [mk(wq_h, wq_v, s)]
            if j == j_uk:
                return [mk(wuk_h, wuk_v, s)]
            if j_ckv <= j < j_uv:
                return [ckv_copy(j - j_ckv)]
            if j == j_uv:
                return [mk(wuv_h, wuv_v, s)]
            if j == j_o:
                return [mk(wo_h, wo_v, s)]
            if j == j_g:
                return [mk(wg_h, wg_v, s)]
            if j == j_u:
                return [mk(wu_h, wu_v, s)]
            if j_d <= j < j_a:
                return [wd_copy(j - j_d)]
            if j == j_a:
                return [mk(wd_h.at[pl.ds(off_a, WD_A)], wd_v.at[pl.ds(off_a, WD_A)], s)]
            assert j == j_v
            return [mk(wd_h.at[pl.ds(off_v, WD_V)], wd_v.at[pl.ds(off_v, WD_V)], s)]

        def start(j):
            if j < n_j:
                for cp in copies(j):
                    cp.start()

        def wait(j):
            for cp in copies(j):
                cp.wait()
            start(j + RING)

        for j in range(RING):
            start(j)

        row128 = jax.lax.broadcasted_iota(jnp.int32, (128, 128), 0)
        col128 = jax.lax.broadcasted_iota(jnp.int32, (128, 128), 1)
        row32 = jax.lax.broadcasted_iota(jnp.int32, (H, 128), 0)
        col32 = jax.lax.broadcasted_iota(jnp.int32, (H, 128), 1)

        def rep_tile(t):
            return jnp.where(row128 == 4 * t + (col128 >> 5), 1.0, 0.0).astype(BF16)

        def rep_tile_t(t):
            return jnp.where(col128 == 4 * t + (row128 >> 5), 1.0, 0.0).astype(BF16)

        def head_mask(v):
            return jnp.where((col32 & (H - 1)) == row32, v, 0.0)

        def layernorm(v):
            mu = jnp.mean(v, axis=-1, keepdims=True)
            ce = v - mu
            var = jnp.mean(ce * ce, axis=-1, keepdims=True)
            return ce * jax.lax.rsqrt(var + 1e-5)

        def stack4(v):
            return jnp.concatenate([v[:, 128 * i:128 * (i + 1)] for i in range(4)], axis=0)

        def head_contract(lhs_stack, w_v):
            def body(t, acc):
                e = jnp.dot(lhs_stack, rep_tile(t), preferred_element_type=F32)
                for i in range(4):
                    a = head_mask(e[H * i:H * (i + 1)]).astype(BF16)
                    off = pl.multiple_of(4096 * i + 128 * t, 128)
                    acc = acc + jnp.dot(a, w_v[pl.ds(off, 128), :], preferred_element_type=F32)
                return acc
            return jax.lax.fori_loop(0, 32, body, jnp.zeros((H, D), F32), unroll=UNROLL_T)

        wait(j_mod)
        cf = c_v[...].astype(F32)
        sc16 = jnp.broadcast_to(cf * jax.nn.sigmoid(cf), (16, M)).astype(BF16)

        def mod_body(i, carry):
            off = pl.multiple_of(i * M, M)
            mod_v[i] = jnp.dot(sc16, wmod_v[:, pl.ds(off, M)], preferred_element_type=F32)[0:8]
            return carry
        jax.lax.fori_loop(0, 6, mod_body, 0)

        def modrow(i):
            return mod_v[i][0:1, :].astype(BF16).astype(F32)

        xf = x_v[...].astype(F32)
        h1 = layernorm(xf) * (1.0 + modrow(1)) + modrow(0)
        h1_stack = stack4(jnp.broadcast_to(h1, (H, M)).astype(BF16))

        wait(j_q)
        qb = head_contract(h1_stack, wq_v).astype(BF16)

        wait(j_uk)
        scale = D ** -0.5

        def ql_body(t, acc):
            zs = []
            for i in range(4):
                off = pl.multiple_of(4096 * i + 128 * t, 128)
                tt = jax.lax.dot_general(qb, wuk_v[pl.ds(off, 128), :], (((1,), (1,)), ((), ())),
                                         preferred_element_type=F32)
                zs.append(head_mask(tt * scale).astype(BF16))
            return acc + jnp.dot(jnp.concatenate(zs, axis=0), rep_tile_t(t), preferred_element_type=F32)
        ql_stack = jax.lax.fori_loop(0, 32, ql_body, jnp.zeros((128, 128), F32), unroll=UNROLL_T)
        ql = jnp.concatenate([ql_stack[H * i:H * (i + 1)] for i in range(4)], axis=1).astype(BF16)

        def attn_body(i, carry):
            m, l, acc = carry
            ckv_copy(i).wait()

            @pl.when(i + RING < n_ckv)
            def _():
                ckv_copy(i + RING).start()

            for r in range(RING):
                @pl.when(i + RING == n_ckv + r)
                def _():
                    start(j_uv + r)

            cc = ckv_v[pl.ds(pl.multiple_of(i * tk, tk), tk), :]
            s = jax.lax.dot_general(ql, cc, (((1,), (1,)), ((), ())), preferred_element_type=F32)
            m_new = jnp.maximum(m, jnp.max(s, axis=1, keepdims=True))
            alpha = jnp.exp(m - m_new)
            p = jnp.exp(s - m_new)
            l = alpha * l + jnp.sum(p, axis=1, keepdims=True)
            acc = alpha * acc + jnp.dot(p.astype(BF16), cc, preferred_element_type=F32)
            return m_new, l, acc

        _, l, acc = jax.lax.fori_loop(
            0, n_ckv, attn_body,
            (jnp.full((H, 1), -jnp.inf, F32), jnp.zeros((H, 1), F32), jnp.zeros((H, DC), F32)))
        o_stack = stack4((acc / l).astype(BF16))

        wait(j_uv)
        ctx = head_contract(o_stack, wuv_v)

        wait(j_o)

        def o_body(hh, acc):
            a = jnp.where(row32 == hh, ctx, 0.0).astype(BF16)
            off = pl.multiple_of(hh * D, D)
            return acc + jnp.dot(a, wo_v[pl.ds(off, D), :], preferred_element_type=F32)
        oacc = jax.lax.fori_loop(0, H, o_body, jnp.zeros((H, M), F32), unroll=UNROLL_H)
        x1 = xf + modrow(2) * jnp.sum(oacc, axis=0, keepdims=True)
        h2 = layernorm(x1) * (1.0 + modrow(4)) + modrow(3)
        h2b = jnp.broadcast_to(h2, (16, M)).astype(BF16)

        wait(j_g)
        g = jnp.dot(h2b, wg_v[...], preferred_element_type=F32)[0:8]
        wait(j_u)
        u = jnp.dot(h2b, wu_v[...], preferred_element_type=F32)[0:8]
        act = jax.nn.gelu(g, approximate=True) * u
        actb = act.astype(BF16)
        for i in range(N_WD):
            act_v[i] = actb[:, WD_CH * i:WD_CH * (i + 1)]
        act_a = actb[:, off_a:off_v]
        acol = jnp.broadcast_to(actb.astype(F32)[0:1, off_v:], (WD_V, 128)).T
        gb8 = jnp.broadcast_to(modrow(5), (8, M))
        x18 = jnp.broadcast_to(x1, (8, M))

        def d_body(i, y):
            wd_copy(i).wait()

            @pl.when(i + RING < N_WD)
            def _():
                wd_copy(i + RING).start()

            for r in range(2):
                @pl.when(i + RING == N_WD + r)
                def _():
                    start(j_a + r)

            off = pl.multiple_of(i * WD_CH, WD_CH)
            return y + jnp.dot(act_v[i], wd_v[pl.ds(off, WD_CH), :], preferred_element_type=F32)[0:8]
        y = jax.lax.fori_loop(0, N_WD, d_body, jnp.zeros((8, M), F32))

        wait(j_a)
        y = y + jnp.dot(act_a, wd_v[pl.ds(off_a, WD_A), :], preferred_element_type=F32)[0:8]
        base = x18 + gb8 * y

        wait(j_v)
        parts = []
        for j in range(M // 128):
            acc_v = None
            for r in range(WD_V // 16):
                w = wd_v[pl.ds(off_v + 16 * r, 16), pl.ds(128 * j, 128)].astype(F32) * acol[16 * r:16 * (r + 1)]
                w = w[0:8] + w[8:16]
                acc_v = w if acc_v is None else acc_v + w
            parts.append(acc_v)
        yv = jnp.sum(jnp.concatenate(parts, axis=1), axis=0, keepdims=True)
        res = base + gb8 * jnp.broadcast_to(yv, (8, M))
        o_ref[...] = res.astype(BF16)[0:1]

    hbm = pl.BlockSpec(memory_space=pltpu.HBM)

    def call(A_x, A_c_kv, A_w_q, A_w_uk, A_w_uv, A_w_o, B_x, B_w_gate, B_w_up, B_w_down, c, w_mod):
        del B_x
        out = pl.pallas_call(
            kernel,
            out_shape=jax.ShapeDtypeStruct((1, M), BF16),
            in_specs=[hbm] * 11,
            out_specs=pl.BlockSpec(memory_space=pltpu.VMEM),
            scratch_shapes=[
                pltpu.VMEM((1, M), BF16), pltpu.VMEM((sk, DC), BF16),
                pltpu.VMEM((M * H, D), BF16), pltpu.VMEM((DC * H, D), BF16), pltpu.VMEM((DC * H, D), BF16),
                pltpu.VMEM((H * D, M), BF16), pltpu.VMEM((M, DF), BF16), pltpu.VMEM((M, DF), BF16),
                pltpu.VMEM((DF, M), BF16), pltpu.VMEM((1, M), BF16), pltpu.VMEM((M, 6 * M), BF16),
                pltpu.VMEM((6, 8, M), F32), pltpu.VMEM((N_WD, 8, WD_CH), BF16),
                pltpu.SemaphoreType.DMA((RING,)),
            ],
            compiler_params=pltpu.CompilerParams(vmem_limit_bytes=100 * 1024 * 1024),
            interpret=interpret,
        )(A_x.reshape(1, M), A_c_kv.reshape(sk, DC), A_w_q.reshape(M * H, D), A_w_uk.reshape(DC * H, D),
          A_w_uv.reshape(DC * H, D), A_w_o.reshape(H * D, M), B_w_gate, B_w_up, B_w_down, c, w_mod)
        return out.reshape(1, 1, M)

    return call


_call = _make()


@jax.jit
def pallas_adaLN_cond__compressed_kv_cla__glu_gated_geglu__decode_kernel(
    A_x: jax.Array,
    A_c_kv: jax.Array,
    A_w_q: jax.Array,
    A_w_uk: jax.Array,
    A_w_uv: jax.Array,
    A_w_o: jax.Array,
    B_x: jax.Array,
    B_w_gate: jax.Array,
    B_w_up: jax.Array,
    B_w_down: jax.Array,
    c: jax.Array,
    w_mod: jax.Array,
):
    return _call(A_x, A_c_kv, A_w_q, A_w_uk, A_w_uv, A_w_o, B_x, B_w_gate, B_w_up, B_w_down, c, w_mod)
```

```python
import jax
import jax.numpy as jnp
from jax.experimental import pallas as pl
from jax.experimental.pallas import tpu as pltpu

F32 = jnp.float32
BF16 = jnp.bfloat16

H, D, M, DC, DF = 32, 128, 512, 512, 1792
SK = 32768
N_CKV = 16
N_WD, WD_CH = 6, 256
WD_A = 128
WD_V = (96, 32)
UNROLL_T, UNROLL_H = 8, 8


def _make(sk=SK, n_ckv=N_CKV, interpret=False):
    tk = sk // n_ckv
    off_a = N_WD * WD_CH
    off_v = off_a + WD_A
    assert tk * n_ckv == sk and off_v + sum(WD_V) == DF and sum(WD_V) == 128

    def kernel(x_h, ckv_h, wq_h, wuk_h, wuv_h, wo_h, wg_h, wu_h, wd_h, c_h, wmod_h, o_ref, *scratch):
        pl.run_scoped(
            lambda sems: body(x_h, ckv_h, wq_h, wuk_h, wuv_h, wo_h, wg_h, wu_h, wd_h, c_h, wmod_h,
                              o_ref, *scratch, sems),
            pltpu.SemaphoreType.DMA((s_end,)))

    s_mod, s_x, s_c, s_q, s_uk, s_ckv = range(6)
    s_uv = s_ckv + n_ckv
    s_o, s_g, s_u, s_d = s_uv + 1, s_uv + 2, s_uv + 3, s_uv + 4
    s_a = s_d + N_WD
    s_v = s_a + 1
    s_end = s_v + len(WD_V)

    def body(x_h, ckv_h, wq_h, wuk_h, wuv_h, wo_h, wg_h, wu_h, wd_h, c_h, wmod_h, o_ref,
             x_v, ckv_v, wq_v, wuk_v, wuv_v, wo_v, wg_v, wu_v, wd_v, c_v, wmod_v, mod_v, act_v, sems):
        def whole(src, dst, s):
            return pltpu.make_async_copy(src, dst, sems.at[s])

        def rows(src, dst, off, n, s):
            return pltpu.make_async_copy(src.at[pl.ds(off, n)], dst.at[pl.ds(off, n)], sems.at[s])

        def ckv_copy(i):
            return rows(ckv_h, ckv_v, pl.multiple_of(i * tk, tk), tk, s_ckv + i)

        def wd_copy(i):
            return rows(wd_h, wd_v, pl.multiple_of(i * WD_CH, WD_CH), WD_CH, s_d + i)

        cp_mod, cp_x, cp_c = whole(wmod_h, wmod_v, s_mod), whole(x_h, x_v, s_x), whole(c_h, c_v, s_c)
        cp_q, cp_uk = whole(wq_h, wq_v, s_q), whole(wuk_h, wuk_v, s_uk)
        cp_uv, cp_o = whole(wuv_h, wuv_v, s_uv), whole(wo_h, wo_v, s_o)
        cp_g, cp_u = whole(wg_h, wg_v, s_g), whole(wu_h, wu_v, s_u)
        cp_a = rows(wd_h, wd_v, off_a, WD_A, s_a)
        v_off = [off_v + sum(WD_V[:k]) for k in range(len(WD_V))]
        cp_v = [rows(wd_h, wd_v, v_off[k], WD_V[k], s_v + k) for k in range(len(WD_V))]

        for cp in (cp_mod, cp_x, cp_c, cp_q, cp_uk):
            cp.start()
        for i in range(n_ckv):
            ckv_copy(i).start()
        for cp in (cp_uv, cp_o, cp_g, cp_u):
            cp.start()
        for i in range(N_WD):
            wd_copy(i).start()
        for cp in (cp_a, *cp_v):
            cp.start()

        row128 = jax.lax.broadcasted_iota(jnp.int32, (128, 128), 0)
        col128 = jax.lax.broadcasted_iota(jnp.int32, (128, 128), 1)
        row32 = jax.lax.broadcasted_iota(jnp.int32, (H, 128), 0)
        col32 = jax.lax.broadcasted_iota(jnp.int32, (H, 128), 1)

        def rep_tile(t):
            return jnp.where(row128 == 4 * t + (col128 >> 5), 1.0, 0.0).astype(BF16)

        def rep_tile_t(t):
            return jnp.where(col128 == 4 * t + (row128 >> 5), 1.0, 0.0).astype(BF16)

        def head_mask(v):
            return jnp.where((col32 & (H - 1)) == row32, v, 0.0)

        def layernorm(v):
            mu = jnp.mean(v, axis=-1, keepdims=True)
            ce = v - mu
            var = jnp.mean(ce * ce, axis=-1, keepdims=True)
            return ce * jax.lax.rsqrt(var + 1e-5)

        def stack4(v):
            return jnp.concatenate([v[:, 128 * i:128 * (i + 1)] for i in range(4)], axis=0)

        def head_contract(lhs_stack, w_v):
            def step(t, acc):
                e = jnp.dot(lhs_stack, rep_tile(t), preferred_element_type=F32)
                for i in range(4):
                    a = head_mask(e[H * i:H * (i + 1)]).astype(BF16)
                    off = pl.multiple_of(4096 * i + 128 * t, 128)
                    acc = acc + jnp.dot(a, w_v[pl.ds(off, 128), :], preferred_element_type=F32)
                return acc
            return jax.lax.fori_loop(0, 32, step, jnp.zeros((H, D), F32), unroll=UNROLL_T)

        cp_mod.wait()
        cp_x.wait()
        cp_c.wait()
        cf = c_v[...].astype(F32)
        sc16 = jnp.broadcast_to(cf * jax.nn.sigmoid(cf), (16, M)).astype(BF16)

        def mod_step(i, carry):
            off = pl.multiple_of(i * M, M)
            mod_v[i] = jnp.dot(sc16, wmod_v[:, pl.ds(off, M)], preferred_element_type=F32)[0:8]
            return carry
        jax.lax.fori_loop(0, 6, mod_step, 0)

        def modrow(i):
            return mod_v[i][0:1, :].astype(BF16).astype(F32)

        xf = x_v[...].astype(F32)
        h1 = layernorm(xf) * (1.0 + modrow(1)) + modrow(0)
        h1_stack = stack4(jnp.broadcast_to(h1, (H, M)).astype(BF16))

        cp_q.wait()
        qb = head_contract(h1_stack, wq_v).astype(BF16)

        cp_uk.wait()
        scale = D ** -0.5

        def ql_step(t, acc):
            zs = []
            for i in range(4):
                off = pl.multiple_of(4096 * i + 128 * t, 128)
                tt = jax.lax.dot_general(qb, wuk_v[pl.ds(off, 128), :], (((1,), (1,)), ((), ())),
                                         preferred_element_type=F32)
                zs.append(head_mask(tt * scale).astype(BF16))
            return acc + jnp.dot(jnp.concatenate(zs, axis=0), rep_tile_t(t), preferred_element_type=F32)
        ql_stack = jax.lax.fori_loop(0, 32, ql_step, jnp.zeros((128, 128), F32), unroll=UNROLL_T)
        ql = jnp.concatenate([ql_stack[H * i:H * (i + 1)] for i in range(4)], axis=1).astype(BF16)

        def attn_step(i, carry):
            m, l, acc = carry
            ckv_copy(i).wait()
            cc = ckv_v[pl.ds(pl.multiple_of(i * tk, tk), tk), :]
            s = jax.lax.dot_general(ql, cc, (((1,), (1,)), ((), ())), preferred_element_type=F32)
            m_new = jnp.maximum(m, jnp.max(s, axis=1, keepdims=True))
            alpha = jnp.exp(m - m_new)
            p = jnp.exp(s - m_new)
            l = alpha * l + jnp.sum(p, axis=1, keepdims=True)
            acc = alpha * acc + jnp.dot(p.astype(BF16), cc, preferred_element_type=F32)
            return m_new, l, acc

        _, l, acc = jax.lax.fori_loop(
            0, n_ckv, attn_step,
            (jnp.full((H, 1), -jnp.inf, F32), jnp.zeros((H, 1), F32), jnp.zeros((H, DC), F32)))
        o_stack = stack4((acc / l).astype(BF16))

        cp_uv.wait()
        ctx = head_contract(o_stack, wuv_v)

        cp_o.wait()

        def o_step(hh, acc):
            a = jnp.where(row32 == hh, ctx, 0.0).astype(BF16)
            off = pl.multiple_of(hh * D, D)
            return acc + jnp.dot(a, wo_v[pl.ds(off, D), :], preferred_element_type=F32)
        oacc = jax.lax.fori_loop(0, H, o_step, jnp.zeros((H, M), F32), unroll=UNROLL_H)
        x1 = xf + modrow(2) * jnp.sum(oacc, axis=0, keepdims=True)
        h2 = layernorm(x1) * (1.0 + modrow(4)) + modrow(3)
        h2b = jnp.broadcast_to(h2, (16, M)).astype(BF16)

        cp_g.wait()
        g = jnp.dot(h2b, wg_v[...], preferred_element_type=F32)[0:8]
        cp_u.wait()
        u = jnp.dot(h2b, wu_v[...], preferred_element_type=F32)[0:8]
        actb = (jax.nn.gelu(g, approximate=True) * u).astype(BF16)
        for i in range(N_WD):
            act_v[i] = actb[:, WD_CH * i:WD_CH * (i + 1)]
        act_a = actb[:, off_a:off_v]
        acol = jnp.broadcast_to(actb.astype(F32)[0:1, off_v:], (128, 128)).T
        gb8 = jnp.broadcast_to(modrow(5), (8, M))
        x18 = jnp.broadcast_to(x1, (8, M))

        def d_step(i, y):
            wd_copy(i).wait()
            off = pl.multiple_of(i * WD_CH, WD_CH)
            return y + jnp.dot(act_v[i], wd_v[pl.ds(off, WD_CH), :], preferred_element_type=F32)[0:8]
        y = jax.lax.fori_loop(0, N_WD, d_step, jnp.zeros((8, M), F32))

        cp_a.wait()
        y = y + jnp.dot(act_a, wd_v[pl.ds(off_a, WD_A), :], preferred_element_type=F32)[0:8]
        base = x18 + gb8 * y

        parts = [None] * (M // 128)
        for k in range(len(WD_V)):
            cp_v[k].wait()
            for j in range(M // 128):
                for r0 in range(v_off[k], v_off[k] + WD_V[k], 16):
                    w = wd_v[pl.ds(r0, 16), pl.ds(128 * j, 128)].astype(F32) * acol[r0 - off_v:r0 - off_v + 16]
                    w = w[0:8] + w[8:16]
                    parts[j] = w if parts[j] is None else parts[j] + w
        yv = jnp.sum(jnp.concatenate(parts, axis=1), axis=0, keepdims=True)
        res = base + gb8 * jnp.broadcast_to(yv, (8, M))
        o_ref[...] = res.astype(BF16)[0:1]

    hbm = pl.BlockSpec(memory_space=pltpu.HBM)

    def call(A_x, A_c_kv, A_w_q, A_w_uk, A_w_uv, A_w_o, B_x, B_w_gate, B_w_up, B_w_down, c, w_mod):
        del B_x
        out = pl.pallas_call(
            kernel,
            out_shape=jax.ShapeDtypeStruct((1, M), BF16),
            in_specs=[hbm] * 11,
            out_specs=pl.BlockSpec(memory_space=pltpu.VMEM),
            scratch_shapes=[
                pltpu.VMEM((1, M), BF16), pltpu.VMEM((sk, DC), BF16),
                pltpu.VMEM((M * H, D), BF16), pltpu.VMEM((DC * H, D), BF16), pltpu.VMEM((DC * H, D), BF16),
                pltpu.VMEM((H * D, M), BF16), pltpu.VMEM((M, DF), BF16), pltpu.VMEM((M, DF), BF16),
                pltpu.VMEM((DF, M), BF16), pltpu.VMEM((1, M), BF16), pltpu.VMEM((M, 6 * M), BF16),
                pltpu.VMEM((6, 8, M), F32), pltpu.VMEM((N_WD, 8, WD_CH), BF16),
            ],
            compiler_params=pltpu.CompilerParams(vmem_limit_bytes=100 * 1024 * 1024),
            interpret=interpret,
        )(A_x.reshape(1, M), A_c_kv.reshape(sk, DC), A_w_q.reshape(M * H, D), A_w_uk.reshape(DC * H, D),
          A_w_uv.reshape(DC * H, D), A_w_o.reshape(H * D, M), B_w_gate, B_w_up, B_w_down, c, w_mod)
        return out.reshape(1, 1, M)

    return call


_call = _make()


@jax.jit
def pallas_adaLN_cond__compressed_kv_cla__glu_gated_geglu__decode_kernel(
    A_x: jax.Array,
    A_c_kv: jax.Array,
    A_w_q: jax.Array,
    A_w_uk: jax.Array,
    A_w_uv: jax.Array,
    A_w_o: jax.Array,
    B_x: jax.Array,
    B_w_gate: jax.Array,
    B_w_up: jax.Array,
    B_w_down: jax.Array,
    c: jax.Array,
    w_mod: jax.Array,
):
    return _call(A_x, A_c_kv, A_w_q, A_w_uk, A_w_uv, A_w_o, B_x, B_w_gate, B_w_up, B_w_down, c, w_mod)
```
